```python
import jax
import jax.numpy as jnp

def _softmax(x, axis=-1):
    return jax.nn.softmax(x, axis=axis)
def _gelu(x):
    return jax.nn.gelu(x, approximate=True)
def _silu(x):
    return jax.nn.silu(x)
def _sigmoid(x):
    return jax.nn.sigmoid(x)
def _layernorm(x, axis=-1, eps=1e-5):
    m = jnp.mean(x, axis=axis, keepdims=True)
    v = jnp.var(x, axis=axis, keepdims=True)
    return (x - m) / jnp.sqrt(v + eps)
def _scatter_add(tgt, idx, src, axis=0):
    return tgt.at[idx].add(src)
def _segment_sum(src, seg, n):
    return jax.ops.segment_sum(src, seg, n)
class _Rng:
    def __init__(self, key):
        self._k = key
    def _next(self):
        self._k, sub = jax.random.split(self._k)
        return sub
    def normal(self, shape):
        return jax.random.normal(self._next(), shape, dtype=jnp.bfloat16)
    def randint(self, lo, hi, shape):
        return jax.random.randint(self._next(), shape, lo, hi, dtype=jnp.int32)
    def uniform(self, shape, lo=0.0, hi=1.0):
        return jax.random.uniform(self._next(), shape, jnp.bfloat16, lo, hi)
    def permutation(self, n):
        return jax.random.permutation(self._next(), n)


kernel_name = 'interleave_layers__sliding_block_cached__glu_gated_glu__decode'

def setup_inputs():
    _rng = _Rng(jax.random.key(int.from_bytes(__import__("os").urandom(4), "little")))
    _w = (lambda a: (lambda t: t.astype(jnp.bfloat16) if jnp.issubdtype(t.dtype, jnp.floating) else t)(jnp.asarray(a)))
    def _A_setup():
        B, Sq, D = 1, 1, 640
        Hq, Hkv, Sk, Dh = 32, 32, 32768, 192
        assert Hq % Hkv == 0, (Hq, Hkv)
        return {
            "x": _w((lambda *s: _rng.normal(s) * 0.05)(B, Sq, D)),
            "k_cache": _w((lambda *s: _rng.normal(s) * 0.05)(B, Hkv, Sk, Dh)),
            "v_cache": _w((lambda *s: _rng.normal(s) * 0.05)(B, Hkv, Sk, Dh)),
            "wq": _w((lambda *s: _rng.normal(s) * 0.05)(D, Hq * Dh) * (D ** -0.5)),
            "wo": _w((lambda *s: _rng.normal(s) * 0.05)(Hq * Dh, D) * ((Hq * Dh) ** -0.5)),
        }
    _A_in = _A_setup()

    def _B_setup():
        B, S, D, F = 1, 1, 640, 1536
        return {
            "x": _w((lambda *s: _rng.normal(s) * 0.05)(B, S, D)),
            "w_gate": _w((lambda *s: _rng.normal(s) * 0.05)(D, F)),
            "w_up": _w((lambda *s: _rng.normal(s) * 0.05)(D, F)),
            "w_down": _w((lambda *s: _rng.normal(s) * 0.05)(F, D)),
        }
    _B_in = _B_setup()

    return {
        "A_x": _A_in["x"],
        "A_k_cache": _A_in["k_cache"],
        "A_v_cache": _A_in["v_cache"],
        "A_wq": _A_in["wq"],
        "A_wo": _A_in["wo"],
        "B_x": _B_in["x"],
        "B_w_gate": _B_in["w_gate"],
        "B_w_up": _B_in["w_up"],
        "B_w_down": _B_in["w_down"],
    }

def reference(A_x, A_k_cache, A_v_cache, A_wq, A_wo, B_x, B_w_gate, B_w_up, B_w_down):
    def _A_ref(x, k_cache, v_cache, wq, wo):
        B, Sq, D = x.shape
        Hq, Dh = 32, 192
        Hkv, Sk = k_cache.shape[1], k_cache.shape[2]
        W = min(4096, max(256, Sk // 4))
        rep = Hq // Hkv
        q = (lambda x, *d: x.transpose(*d))((x @ wq).reshape(B, Sq, Hq, Dh), 0, 2, 1, 3)
        k = jnp.repeat(k_cache[:, :, Sk - W:, :], rep, axis=1)
        v = jnp.repeat(v_cache[:, :, Sk - W:, :], rep, axis=1)
        scores = jnp.einsum("bhqd,bhkd->bhqk", q, k) * (Dh ** -0.5)
        p = _softmax(scores, axis=-1)
        o = jnp.einsum("bhqk,bhkd->bhqd", p, v)
        return (lambda x, *d: x.transpose(*d))(o, 0, 2, 1, 3).reshape(B, Sq, Hq * Dh) @ wo

    def _B_ref(x, w_gate, w_up, w_down):
        g = jnp.einsum("bsd,df->bsf", x, w_gate)
        u = jnp.einsum("bsd,df->bsf", x, w_up)
        h = _sigmoid(g) * u
        return jnp.einsum("bsf,fd->bsd", h, w_down)

    x = A_x
    x = x + _A_ref(_layernorm(x, axis=-1), A_k_cache, A_v_cache, A_wq, A_wo)
    x = x + _B_ref(_layernorm(x, axis=-1), B_w_gate, B_w_up, B_w_down)
    x = x + _A_ref(_layernorm(x, axis=-1), A_k_cache, A_v_cache, A_wq, A_wo)
    x = x + _B_ref(_layernorm(x, axis=-1), B_w_gate, B_w_up, B_w_down)
    return x
```

```python
import functools

import jax
import jax.numpy as jnp
import numpy as np
from jax.experimental import pallas as pl
from jax.experimental.pallas import tpu as pltpu

_HQ = 32
_DH = 192
_HG = 8
_LANES = 128
_EPS = 1e-5
_LOG2E = 1.4426950408889634


def _layernorm(x):
    m = jnp.mean(x, axis=-1, keepdims=True)
    d = x - m
    v = jnp.mean(d * d, axis=-1, keepdims=True)
    return d * jax.lax.rsqrt(v + _EPS)


def _dot(a, b):
    return jnp.dot(a, b, preferred_element_type=jnp.float32)


def _kernel(x_hbm, k_hbm, v_hbm, wq_hbm, wo_hbm, wg_hbm, wu_hbm, wd_hbm, o_ref,
            xbuf, kbuf, vbuf, wq, wo, wg, wu, wd, qbd, s_ref, p_ref, o_acc,
            kv_sems, w_sems, *, start, depth):
    nc = kbuf.shape[0]
    rows = _HG * _DH
    ng = _HQ // _HG
    d_model = xbuf.shape[-1]
    c2 = (_DH ** -0.5) * _LOG2E

    def k_copy(c):
        return pltpu.make_async_copy(
            k_hbm.at[:, pl.ds(pl.multiple_of(start + c * _LANES, _LANES), _LANES)],
            kbuf.at[c], kv_sems.at[0, c])

    def v_copy(c):
        return pltpu.make_async_copy(
            v_hbm.at[:, pl.ds(pl.multiple_of(start + c * _LANES, _LANES), _LANES)],
            vbuf.at[c], kv_sems.at[1, c])

    x_copy = pltpu.make_async_copy(x_hbm, xbuf, w_sems.at[0])
    wq_copy = pltpu.make_async_copy(wq_hbm, wq, w_sems.at[1])
    wo_copy = pltpu.make_async_copy(wo_hbm, wo, w_sems.at[2])
    wg_copy = pltpu.make_async_copy(wg_hbm, wg, w_sems.at[3])
    wu_copy = pltpu.make_async_copy(wu_hbm, wu, w_sems.at[4])
    wd_copy = pltpu.make_async_copy(wd_hbm, wd, w_sems.at[5])

    col = jax.lax.broadcasted_iota(jnp.int32, (_HG, rows), 1)
    lo = jax.lax.broadcasted_iota(jnp.int32, (_HG, rows), 0) * _DH
    diag = (col >= lo) & (col < lo + _DH)

    def q_group(xn, g):
        q = _dot(xn, wq[:, g * rows:(g + 1) * rows])
        return jnp.where(diag, q, 0.0).astype(jnp.bfloat16)

    def softmax_group(s_tiles):
        m = functools.reduce(jnp.maximum, s_tiles)
        m = jnp.max(m, axis=-1, keepdims=True)
        p_tiles = [jnp.exp2((s - m) * c2) for s in s_tiles]
        l = functools.reduce(jnp.add, p_tiles)
        l = jnp.sum(l, axis=-1, keepdims=True)
        return [p.astype(jnp.bfloat16) for p in p_tiles], l

    def pv_tile(p, c, g):
        return [_dot(p, vbuf[c, pl.ds(g * rows + t * _LANES, _LANES), :])
                for t in range(rows // _LANES)]

    def out_group(o, l, g):
        o = jnp.where(diag, o, 0.0) * (1.0 / l)
        return _dot(o.astype(jnp.bfloat16), wo[g * rows:(g + 1) * rows, :])

    def glu(xn, wait):
        if wait:
            wg_copy.wait()
        gate = _dot(xn, wg[...])
        if wait:
            wu_copy.wait()
        up = _dot(xn, wu[...])
        h = (jax.nn.sigmoid(gate) * up).astype(jnp.bfloat16)
        if wait:
            wd_copy.wait()
        return _dot(h, wd[...])

    def rowsum(a):
        return jnp.broadcast_to(jnp.sum(a, axis=0, keepdims=True), a.shape)

    x_copy.start()
    wq_copy.start()
    for c in range(depth):
        k_copy(c).start()

    x_copy.wait()
    x = jnp.broadcast_to(xbuf[0].astype(jnp.float32), (_HG, d_model))
    xn = _layernorm(x).astype(jnp.bfloat16)
    wq_copy.wait()
    for g in range(ng):
        qbd[g] = q_group(xn, g)

    def k_step(c, carry):
        k_copy(c).wait()

        @pl.when(c + depth < nc)
        def _():
            k_copy(c + depth).start()

        @pl.when(c + depth >= nc)
        def _():
            v_copy(c + depth - nc).start()

        for g in range(ng):
            s_ref[g, c] = _dot(qbd[g], kbuf[c, g * rows:(g + 1) * rows, :])
        return carry

    jax.lax.fori_loop(0, nc, k_step, 0)

    ls = []
    for g in range(ng):
        p_tiles, l = softmax_group([s_ref[g, c] for c in range(nc)])
        for c in range(nc):
            p_ref[g, c] = p_tiles[c]
        ls.append(l)
    o_acc[...] = jnp.zeros(o_acc.shape, jnp.float32)

    def v_step(c, carry):
        v_copy(c).wait()

        @pl.when(c + depth < nc)
        def _():
            v_copy(c + depth).start()

        @pl.when(c + depth == nc)
        def _():
            wo_copy.start()
            wg_copy.start()
            wu_copy.start()
            wd_copy.start()

        for t in range(ng * rows // _LANES):
            sl = pl.ds(t * _LANES, _LANES)
            vbuf[c, sl, :] = vbuf[c, sl, :].T
        for g in range(ng):
            o_acc[g] += jnp.concatenate(pv_tile(p_ref[g, c], c, g), axis=1)
        return carry

    jax.lax.fori_loop(0, nc, v_step, 0)

    wo_copy.wait()
    a = functools.reduce(jnp.add, [out_group(o_acc[g], ls[g], g) for g in range(ng)])
    x = x + rowsum(a)
    x = x + glu(_layernorm(x).astype(jnp.bfloat16), True)

    xn = _layernorm(x).astype(jnp.bfloat16)
    outs = []
    for g in range(ng):
        q = q_group(xn, g)
        s_tiles = [_dot(q, kbuf[c, g * rows:(g + 1) * rows, :]) for c in range(nc)]
        p_tiles, l = softmax_group(s_tiles)
        acc = None
        for c in range(nc):
            r = pv_tile(p_tiles[c], c, g)
            acc = r if acc is None else [u + w for u, w in zip(acc, r)]
        outs.append(out_group(jnp.concatenate(acc, axis=1), l, g))
    x = x + rowsum(functools.reduce(jnp.add, outs))
    x = x + glu(_layernorm(x).astype(jnp.bfloat16), False)
    o_ref[0] = x[0:1, :].astype(o_ref.dtype)


@jax.jit
def pallas_interleave_layers__sliding_block_cached__glu_gated_glu__decode_kernel(
    A_x: jax.Array,
    A_k_cache: jax.Array,
    A_v_cache: jax.Array,
    A_wq: jax.Array,
    A_wo: jax.Array,
    B_x: jax.Array,
    B_w_gate: jax.Array,
    B_w_up: jax.Array,
    B_w_down: jax.Array,
):
    del B_x
    _, hkv, sk, dh = A_k_cache.shape
    assert A_x.shape[:2] == (1, 1) and hkv == _HQ and dh == _DH
    window = min(4096, max(256, sk // 4))
    assert window % _LANES == 0 and (sk - window) % _LANES == 0
    nc = window // _LANES
    ng = _HQ // _HG
    rows = _HG * _DH
    bf16 = jnp.bfloat16

    kt = jnp.transpose(A_k_cache, (0, 1, 3, 2)).reshape(hkv * dh, sk)
    vt = jnp.transpose(A_v_cache, (0, 1, 3, 2)).reshape(hkv * dh, sk)

    hbm = pl.BlockSpec(memory_space=pltpu.HBM)
    return pl.pallas_call(
        functools.partial(_kernel, start=sk - window, depth=min(4, nc)),
        out_shape=jax.ShapeDtypeStruct(A_x.shape, A_x.dtype),
        in_specs=[hbm] * 8,
        out_specs=pl.BlockSpec(memory_space=pltpu.VMEM),
        scratch_shapes=[
            pltpu.VMEM(A_x.shape, bf16),
            pltpu.VMEM((nc, hkv * dh, _LANES), bf16),
            pltpu.VMEM((nc, hkv * dh, _LANES), bf16),
            pltpu.VMEM(A_wq.shape, bf16),
            pltpu.VMEM(A_wo.shape, bf16),
            pltpu.VMEM(B_w_gate.shape, bf16),
            pltpu.VMEM(B_w_up.shape, bf16),
            pltpu.VMEM(B_w_down.shape, bf16),
            pltpu.VMEM((ng, _HG, rows), bf16),
            pltpu.VMEM((ng, nc, _HG, _LANES), jnp.float32),
            pltpu.VMEM((ng, nc, _HG, _LANES), bf16),
            pltpu.VMEM((ng, _HG, rows), jnp.float32),
            pltpu.SemaphoreType.DMA((2, nc)),
            pltpu.SemaphoreType.DMA((6,)),
        ],
        compiler_params=pltpu.CompilerParams(vmem_limit_bytes=127 * 1024 * 1024),
    )(A_x, kt, vt, A_wq, A_wo, B_w_gate, B_w_up, B_w_down)
```

```python
import functools

import jax
import jax.numpy as jnp
import numpy as np
from jax.experimental import pallas as pl
from jax.experimental.pallas import tpu as pltpu

_HQ = 32
_DH = 192
_L = 128
_EPS = 1e-5
_C2 = (_DH ** -0.5) * 1.4426950408889634

CFG = dict(groups=(2, 2, 4, 4, 6, 8, 6), n_mxu=6, nb=4, rb=4, kt=6, lag=250, rlag=0, smlat=200, smd=170, ti=-2, vop=0.27, depth=4, nwd=4, lnt=1, fin=30, mres=2)

f32, bf16, i32 = jnp.float32, jnp.bfloat16, jnp.int32


def _layernorm(x):
    m = jnp.mean(x, axis=-1, keepdims=True)
    d = x - m
    v = jnp.mean(d * d, axis=-1, keepdims=True)
    return d * jax.lax.rsqrt(v + _EPS)


def _lhs(a):
    return jnp.concatenate([a, jnp.zeros_like(a)], axis=0).astype(bf16)


def _dot(a, b):
    return jnp.dot(a, b, preferred_element_type=f32)[0:8]


def _dot_nt(a, b):
    return jax.lax.dot_general(a, b, (((1,), (1,)), ((), ())), preferred_element_type=f32)[0:8]


def _tree(xs, op=jnp.add):
    while len(xs) > 1:
        xs = [op(xs[i], xs[i + 1]) if i + 1 < len(xs) else xs[i] for i in range(0, len(xs), 2)]
    return xs[0]


def _rowsum(a):
    return jnp.broadcast_to(jnp.sum(a, axis=0, keepdims=True), a.shape)


def _softmax(s_tiles):
    m = jnp.max(_tree(s_tiles, jnp.maximum), axis=-1, keepdims=True)
    p_tiles = [jnp.exp2(s - m) for s in s_tiles]
    l = jnp.sum(_tree(p_tiles), axis=-1, keepdims=True)
    return p_tiles, jnp.broadcast_to(1.0 / l, (8, _L))


def _cat(xs):
    return xs[0] if len(xs) == 1 else jnp.concatenate(xs, axis=1)


def _b16(w):
    return pltpu.bitcast(w, bf16)


def _kernel(x_hbm, k_hbm, v_hbm, wq_hbm, wo_hbm, wg_hbm, wu_hbm, wd_hbm, o_ref,
            xbuf, kbuf, vbuf, wq, wo, wg, wu, wd, qbd, s_ref, p_ref, pb, il_ref, o_acc, pk_ref, pbc, dmask,
            kv_sems, w_sems, *, start, cfg):
    nc = kbuf.shape[0]
    d_model = xbuf.shape[-1]
    nd = d_model // _L
    depth = cfg["depth"]
    h_mxu = _HQ - cfg["n_mxu"]
    nwd = cfg["nwd"]
    fc = wd.shape[0] // nwd
    k32, v32, wq32, wo32, qbd32, pb32 = (r.bitcast(i32) for r in (kbuf, vbuf, wq, wo, qbd, pb))

    def k_copy(c):
        return pltpu.make_async_copy(
            k_hbm.at[:, pl.ds(pl.multiple_of(start + c * _L, _L), _L)], kbuf.at[c], kv_sems.at[0, c])

    def v_copy(c):
        return pltpu.make_async_copy(
            v_hbm.at[:, pl.ds(pl.multiple_of(start + c * _L, _L), _L)], vbuf.at[c], kv_sems.at[1, c])

    def wq_copy(t):
        return pltpu.make_async_copy(
            wq_hbm.at[:, pl.ds(pl.multiple_of(t * _L, _L), _L)], wq.at[t], w_sems.at[1])

    def wo_copy(b, t):
        n = wo.shape[1] // nc
        rs = pl.ds(pl.multiple_of(b * n, n), n)
        return pltpu.make_async_copy(wo_hbm.at[rs, pl.ds(t * _L, _L)], wo.at[t, rs], w_sems.at[2])

    x_copy = pltpu.make_async_copy(x_hbm, xbuf, w_sems.at[0])
    wg_copy = pltpu.make_async_copy(wg_hbm, wg, w_sems.at[3])
    wu_copy = pltpu.make_async_copy(wu_hbm, wu, w_sems.at[4])
    wd_copies = [pltpu.make_async_copy(wd_hbm.at[pl.ds(i * fc, fc)], wd.at[pl.ds(i * fc, fc)], w_sems.at[5 + i])
                 for i in range(nwd)]

    def ln_dot(x):
        m = jnp.mean(x, axis=-1, keepdims=True)
        d = x - m
        r = jax.lax.rsqrt(jnp.mean(d * d, axis=-1, keepdims=True) + _EPS)
        xo = jnp.concatenate([x, jnp.ones_like(x)], axis=0).astype(bf16)

        def f(w):
            y = jnp.dot(xo, w, preferred_element_type=f32)
            return (y[0:8] - m * y[8:16]) * r
        return f, _lhs(d * r)

    def put(ref32, a, t0=0, m0=0):
        a = pltpu.bitcast(_lhs(a), i32)
        for t in range(a.shape[1] // _L):
            ref32[t0 + t] = a[:, t * _L:(t + 1) * _L] & dmask[m0 + t]

    k_copy(0).start()
    x_copy.start()

    @pl.loop(0, wq.shape[0])
    def _(t):
        wq_copy(t).start()

    for c in range(1, depth):
        k_copy(c).start()

    for t in range(dmask.shape[0]):
        col = jax.lax.broadcasted_iota(i32, (8, _L), 1) + t * _L
        col = col - jax.lax.broadcasted_iota(i32, (8, _L), 0) * (2 * _DH)
        dmask[t] = jnp.where((col >= 0) & (col < 2 * _DH), jnp.where(col < _DH, 0xFFFF, -65536), 0)
    o_acc[...] = jnp.zeros(o_acc.shape, f32)
    x_copy.wait()
    x = jnp.broadcast_to(xbuf[0].astype(f32), (8, d_model))
    xn = _lhs(_layernorm(x))
    pltpu.make_async_copy(wq, wq, w_sems.at[1]).wait()
    r8 = 8 * _DH
    t8 = r8 // _L

    @pl.loop(0, _HQ // 8)
    def _(g):
        w = wq32.at[pl.ds(g * t8, t8)]
        put(qbd32.at[pl.ds(g * t8, t8)], _dot(xn, _cat([_b16(w[t]) for t in range(t8)])) * _C2)

    def k_step(c, carry):
        k_copy(c).wait()
        for t in range(nd):
            wo_copy(c, t).start()

        @pl.when(c + depth < nc)
        def _():
            k_copy(c + depth).start()

        @pl.when(c + depth >= nc)
        def _():
            v_copy(c + depth - nc).start()

        for g in range(_HQ // 8):
            q = _cat([qbd[g * t8 + t] for t in range(t8)])
            s_ref[g, c] = _dot(q, _b16(k32[c, pl.ds(g * r8 // 2, r8 // 2), :]))
        return carry

    jax.lax.fori_loop(0, nc, k_step, 0)

    @pl.loop(0, _HQ // 8)
    def _(g):
        p_tiles, il_ref[g] = _softmax([s_ref[g, c] for c in range(nc)])
        for c in range(nc):
            s_ref[g, c] = p_tiles[c]

    def v_step(c, carry):
        v_copy(c).wait()

        @pl.when(c + depth < nc)
        def _():
            v_copy(c + depth).start()

        @pl.when(c + depth == nc)
        def _():
            wg_copy.start()
            wu_copy.start()
            for cp in wd_copies:
                cp.start()

        for g in range(_HQ // 8):
            o_acc[g] += _dot_nt(_lhs(s_ref[g, c]), _b16(v32[c, pl.ds(g * r8 // 2, r8 // 2), :]))

        for r0 in range(h_mxu * _DH, _HQ * _DH, _L):
            vbuf[c, pl.ds(r0, _L), :] = vbuf[c, pl.ds(r0, _L), :].T
        return carry + 1

    never = jax.lax.fori_loop(0, nc, v_step, 0) < 0

    pltpu.make_async_copy(wo, wo, w_sems.at[2]).wait()

    def o_step(g, a):
        put(qbd32, o_acc[g] * _cat([il_ref[g]] * t8))
        o = _cat([qbd[t] for t in range(t8)])
        w = wo32.at[:, pl.ds(pl.multiple_of(g * (r8 // 2), r8 // 2), r8 // 2), :]
        return a + _dot(o, _cat([_b16(w[t]) for t in range(nd)]))

    x = x + _rowsum(jax.lax.fori_loop(0, _HQ // 8, o_step, jnp.zeros((8, d_model), f32)))
    xn = _lhs(_layernorm(x))
    wg_copy.wait()
    gate = _dot(xn, wg[...])
    wu_copy.wait()
    hid = _lhs(jax.nn.sigmoid(gate) * _dot(xn, wu[...]))
    for i, cp in enumerate(wd_copies):
        cp.wait()
        x = x + _dot(hid[:, i * fc:(i + 1) * fc], wd[i * fc:(i + 1) * fc, :])

    xn_dot, xn = ln_dot(x)
    groups, lag, rb = cfg["groups"], cfg["lag"], cfg["rb"]
    first = [sum(groups[:g]) for g in range(len(groups))]
    grp = {h: g for g in range(len(groups)) for h in range(first[g], first[g] + groups[g])}
    ones = jnp.ones((16, _L), bf16)
    events, tokens, vhist = [], [], []
    st = {}
    t_q, t_soft, t_head = {}, {}, {}

    def after(a, dep):
        return jnp.where(never, pltpu.bitcast(dep, a.dtype), a)

    def at(t, fn):
        events.append((t, len(events), fn))

    def mxu(tm, cycles, fn):
        def run():
            r = fn()
            tokens.append((tm + cycles + lag, r[:, r.shape[1] - _L:]))
        at(tm, run)
        return tm + cycles

    def lhs_tiles(ref32, t0, n, tm):
        tiles = [ref32[t] for t in range(t0, t0 + n)]
        for v in [v for (t, v) in vhist if t <= tm - cfg["rlag"]][-1:]:
            tiles[0] = after(tiles[0], v)
        return _cat([_b16(u) for u in tiles])

    def put_pair(a, h):
        put(qbd32, a, h // 2 * 3, (h - first[grp[h]]) // 2 * 3)

    tm = 0.0
    q_next = 0
    for g, n in enumerate(groups):
        h0 = first[g]
        nt = n * _DH // _L
        gq = min(g + 1, len(groups) - 1)
        while q_next < first[gq] + groups[gq]:
            def qjob(h=q_next):
                w = _cat([_b16(wq32[t]) for t in range(h // 2 * 3, h // 2 * 3 + 3)])
                q = xn_dot(w) if h < 2 * cfg["lnt"] else _dot(xn, w)
                put_pair(q * _C2, h)
                return q
            tm = mxu(tm, 8 * 3 * nd, qjob)
            t_q[q_next] = tm + 150
            q_next += 2
        tm = max(tm, t_q[h0 + n - 2])
        kt = max(k for k in range(1, cfg["kt"] + 1) if nt % k == 0)
        cn = cfg["kt"] // kt
        for c0 in range(0, nc, cn):
            for t in range(0, nt, kt):
                def kjob(g=g, h0=h0, nt=nt, kt=kt, c0=c0, cn=cn, t=t, tm=tm):
                    rs = pl.ds((h0 * _DH + t * _L) // 2, kt * _L // 2)
                    s = _dot(lhs_tiles(qbd32, h0 // 2 * 3 + t, kt, tm),
                             _cat([_b16(k32[c, rs, :]) for c in range(c0, c0 + cn)]))
                    st["s"] = s = st["s"] + s if t else s
                    if t + kt == nt:
                        for u in range(cn):
                            s_ref[g % 2, c0 + u] = s[:, u * _L:(u + 1) * _L]
                    return s
                tm = mxu(tm, 8 * kt * cn, kjob)

        t, d = tm + lag, cfg["smd"]

        def row_max(g=g, t=t):
            m = jnp.max(_tree([s_ref[g % 2, c] for c in range(nc)], jnp.maximum), axis=-1, keepdims=True)
            st["m", g] = jnp.broadcast_to(m, (8, _L))
            tokens.append((t + d, st["m", g]))
        at(t, row_max)
        for c0 in range(0, nc, 8):
            def exps(g=g, c0=c0, t=t):
                ps = [jnp.exp2(s_ref[g % 2, c] - st["m", g]) for c in range(c0, c0 + 8)]
                for c, p in zip(range(c0, c0 + 8), ps):
                    if first[g] < h_mxu:
                        p_ref[g, c] = p
                    if first[g] + groups[g] > h_mxu:
                        pb[c] = _lhs(p)
                st["l", g] = _tree(ps + ([st["l", g]] if c0 else []))
                tokens.append((t + d + 40 + 3 * c0, st["l", g]))
            at(t + min(d + 3 * c0, cfg["smlat"] - 1), exps)

        def row_sum(g=g):
            il_ref[g] = jnp.broadcast_to(1.0 / jnp.sum(st["l", g], axis=-1, keepdims=True), (8, _L))
        at(t + d + 3 * nc + 40, row_sum)
        t_soft[g] = t + cfg["smlat"]

    tv = 0.0
    nb = cfg["nb"]
    for h in range(h_mxu):
        g = grp[h]
        early = min(60, max(0, tv - t_soft[g]))
        tv = max(tv, t_soft[g])

        def bjob(h=h, g=g):
            for c in range(nc):
                pbc[h % 2, c] = jnp.broadcast_to(p_ref[g, c, pl.ds(h - first[g], 1), :], (8, _L))
        at(tv - early, bjob)
        for r0 in range(0, _DH // 16, rb):
            for b in range(nb):
                c0, c1 = nc * b // nb, nc * (b + 1) // nb

                def pjob(h=h, c0=c0, c1=c1):
                    st["p"] = [pbc[h % 2, c] for c in range(c0, c1)]
                at(tv, pjob)
                for r in range(r0, r0 + rb):
                    def vjob(h=h, c0=c0, c1=c1, r=r, tv=tv):
                        sl = pl.ds(h * (_DH // 2) + r * 8, 8)
                        k = cfg["ti"] % (c1 - c0)
                        los, his = [], []
                        for i, p in enumerate(st["p"]):
                            w = v32[c0 + i, sl, :]
                            if i == k:
                                for _, v in vhist[-1:]:
                                    w = after(w, v)
                                for t, m in tokens:
                                    if t_soft[0] + 50 < t <= tv:
                                        w = after(w, m)
                                tokens[:] = [m for m in tokens if m[0] > tv]
                            los.append(pltpu.bitcast(w << 16, f32) * p)
                            his.append(pltpu.bitcast(w & (-65536), f32) * p)
                        if c0:
                            los.insert(0, st[r][0])
                            his.insert(0, st[r][1])
                            k += 1
                        lo = functools.reduce(jnp.add, ([_tree(los[:k])] if k else []) + los[k:])
                        hi = functools.reduce(jnp.add, ([_tree(his[:k])] if k else []) + his[k:])
                        st[r] = (lo, hi)
                        if c1 < nc:
                            tok = after(hi, lo)
                        else:
                            tok = pltpu.bitcast(pltpu.pack_elementwise([lo, hi], packed_dtype=bf16), i32)
                            pk_ref[sl, :] = tok
                        vhist[:] = vhist[-100:] + [(tv, tok)]
                    at(tv, vjob)
                    tv += (6 * (c1 - c0) + 2) * cfg["vop"]
        t_head[h] = tv

    todo_r = list(range(0, h_mxu, 2))
    todo_m = [(h, c0) for h in range(h_mxu, _HQ, 2) for c0 in range(0, nc, 2)]
    todo_o = []
    while todo_r or todo_m or todo_o:
        m_ok = todo_m and t_soft[grp[todo_m[0][0]]] <= tm
        if todo_r and t_head[todo_r[0] + 1] + cfg["fin"] <= tm:
            h = todo_r.pop(0)

            def rjob(h=h):
                o = _dot_nt(ones, _b16(pk_ref[pl.ds(h * (_DH // 2), _DH), :]))
                put_pair(o * _cat([il_ref[grp[h]]] * 3), h)
                return o
            tm = mxu(tm, 48, rjob)
            todo_o.append((tm + 200, h))
        elif m_ok and (len(todo_o) <= cfg["mres"] or todo_o[0][0] > tm):
            h, c0 = todo_m.pop(0)

            def mjob(h=h, c0=c0, tm=tm):
                for c in range(c0, c0 + 2):
                    r = _dot(lhs_tiles(pb32, c, 1, tm if c == c0 else -1e9),
                             _cat([_b16(v32[c, pl.ds((h * _DH + u * _L) // 2, _L // 2), :]) for u in range(3)]))
                    st["s"] = st["s"] + r if c else r
                if c0 + 2 == nc:
                    put_pair(st["s"] * _cat([il_ref[grp[h]]] * 3), h)
                return st["s"]
            tm = mxu(tm, 48, mjob)
            if c0 + 2 == nc:
                todo_o.append((tm + 200, h))
        elif todo_o and todo_o[0][0] <= tm:
            def ojob(h=todo_o.pop(0)[1], tm=tm):
                y = _dot(lhs_tiles(qbd32, h // 2 * 3, 3, tm),
                         _cat([_b16(wo32[t, pl.ds(h * (_DH // 2), _DH), :]) for t in range(nd)]))
                st["out"] = st["out"] + y if "out" in st else y
                return st["out"]
            tm = mxu(tm, 8 * 3 * nd, ojob)
        else:
            tm += 8

    for _, _, fn in sorted(events, key=lambda e: e[:2]):
        fn()

    x = x + _rowsum(st["out"])
    xn_dot, xn = ln_dot(x)
    if cfg["lnt"]:
        gate, up = xn_dot(wg[...]), xn_dot(wu[...])
    else:
        gate, up = _dot(xn, wg[...]), _dot(xn, wu[...])
    x = x + _dot(_lhs(jax.nn.sigmoid(gate) * up), wd[...])
    o_ref[0] = x[0:1, :].astype(o_ref.dtype)


@jax.jit
def pallas_interleave_layers__sliding_block_cached__glu_gated_glu__decode_kernel(
    A_x, A_k_cache, A_v_cache, A_wq, A_wo, B_x, B_w_gate, B_w_up, B_w_down,
):
    del B_x
    _, hkv, sk, dh = A_k_cache.shape
    d_model = A_x.shape[-1]
    assert A_x.shape[:2] == (1, 1) and hkv == _HQ and dh == _DH
    window = min(4096, max(256, sk // 4))
    assert window % _L == 0 and (sk - window) % _L == 0
    nc = window // _L
    hd = hkv * dh
    ngr = max(hkv // 8, len(CFG["groups"]))

    kt = jnp.transpose(A_k_cache, (0, 1, 3, 2)).reshape(hd, sk)
    vt = jnp.transpose(A_v_cache, (0, 1, 3, 2)).reshape(hd, sk)

    hbm = pl.BlockSpec(memory_space=pltpu.HBM)
    out = pl.pallas_call(
        functools.partial(_kernel, start=sk - window, cfg=CFG),
        out_shape=jax.ShapeDtypeStruct(A_x.shape, A_x.dtype),
        in_specs=[hbm] * 8,
        out_specs=pl.BlockSpec(memory_space=pltpu.VMEM),
        scratch_shapes=[
            pltpu.VMEM(A_x.shape, bf16),
            pltpu.VMEM((nc, hd, _L), bf16),
            pltpu.VMEM((nc, hd, _L), bf16),
            pltpu.VMEM((hd // _L, d_model, _L), bf16),
            pltpu.VMEM((d_model // _L, hd, _L), bf16),
            pltpu.VMEM(B_w_gate.shape, bf16),
            pltpu.VMEM(B_w_up.shape, bf16),
            pltpu.VMEM(B_w_down.shape, bf16),
            pltpu.VMEM((hd // _L, 16, _L), bf16),
            pltpu.VMEM((hkv // 8, nc, 8, _L), f32),
            pltpu.VMEM((ngr, nc, 8, _L), f32),
            pltpu.VMEM((nc, 16, _L), bf16),
            pltpu.VMEM((ngr, 8, _L), f32),
            pltpu.VMEM((hkv // 8, 8, 8 * dh), f32),
            pltpu.VMEM((hd // 2, _L), i32),
            pltpu.VMEM((2, nc, 8, _L), f32),
            pltpu.VMEM((8 * dh // _L, 8, _L), i32),
            pltpu.SemaphoreType.DMA((2, nc)),
            pltpu.SemaphoreType.DMA((5 + CFG["nwd"],)),
        ],
        compiler_params=pltpu.CompilerParams(vmem_limit_bytes=127 * 1024 * 1024),
    )(A_x, kt, vt, A_wq, A_wo, B_w_gate, B_w_up, B_w_down)
    return out
```

```python
import functools

import jax
import jax.numpy as jnp
from jax.experimental import pallas as pl
from jax.experimental.pallas import tpu as pltpu

f32, bf16, i32 = jnp.float32, jnp.bfloat16, jnp.int32

_HQ = 32
_DH = 192
_L = 128
_EPS = 1e-5
_QSCALE = (_DH ** -0.5) * 1.4426950408889634
_HI = -65536
_RING = 4

_GROUPS = (2, 2, 4, 4, 6, 8, 6)
_H_MXU = 26
_C_SPLIT = 16
_C_BLOCK = 8
_R_BLOCK = 4
_WIDE = (0, 1, 8, 9, 16, 24)
_T_TILE = 8
_T_VOP = 0.27
_T_MXU = 200
_T_MAX = 170
_T_SOFTMAX = 200


def _cat(xs):
    return xs[0] if len(xs) == 1 else jnp.concatenate(xs, axis=1)


def _tree(xs, op=jnp.add):
    while len(xs) > 1:
        xs = [op(xs[i], xs[i + 1]) if i + 1 < len(xs) else xs[i] for i in range(0, len(xs), 2)]
    return xs[0]


def _b16(w):
    return pltpu.bitcast(w, bf16)


def _lhs(a):
    return jnp.concatenate([a, jnp.zeros_like(a)], axis=0).astype(bf16)


def _dot(a, b):
    return jnp.dot(a, b, preferred_element_type=f32)[0:8]


def _dot_nt(a, b):
    return jax.lax.dot_general(a, b, (((1,), (1,)), ((), ())), preferred_element_type=f32)[0:8]


def _rowsum(a):
    return jnp.broadcast_to(jnp.sum(a, axis=0, keepdims=True), a.shape)


def _ln_stats(x):
    m = jnp.mean(x, axis=-1, keepdims=True)
    d = x - m
    return m, d, jax.lax.rsqrt(jnp.mean(d * d, axis=-1, keepdims=True) + _EPS)


def _layernorm(x):
    _, d, r = _ln_stats(x)
    return _lhs(d * r)


def _layernorm_dot(x):
    m, d, r = _ln_stats(x)
    x_ones = jnp.concatenate([x, jnp.ones_like(x)], axis=0).astype(bf16)

    def f(w):
        y = jnp.dot(x_ones, w, preferred_element_type=f32)
        return (y[0:8] - m * y[8:16]) * r

    return f, _lhs(d * r)


def _second_attention(q_dot, xn, never, k32, v32, v_lo, wq32, wo32, lhs32, put, s_ref, p_ref, p16,
                      p_row, inv_l, o_acc):
    nc, nd = k32.shape[0], wo32.shape[0]
    p16_32 = p16.bitcast(i32)
    h_vpu = _H_MXU + 2
    first = [sum(_GROUPS[:g]) for g in range(len(_GROUPS))]
    group = [g for g, n in enumerate(_GROUPS) for _ in range(n)]
    assert len(group) == _HQ and group[_H_MXU] == group[-1] and _C_SPLIT < nc
    ones = jnp.ones((16, _L), bf16)
    events = []
    results = []
    steps = []
    st = {}
    t_q, t_soft, t_head = {}, {}, {}

    def after(a, dep):
        return jnp.where(never, pltpu.bitcast(dep, a.dtype), a)

    def at(t, fn):
        events.append((t, len(events), fn))

    def mxu(t, cycles, fn):
        def run():
            r = fn()
            results.append((t + cycles + _T_MXU, r[:, r.shape[1] - _L:]))
        at(t, run)
        return t + cycles

    def lhs_tiles(ref32, t0, n, t):
        tiles = [ref32[i] for i in range(t0, t0 + n)]
        for v in [v for (tv, v) in steps if tv <= t][-1:]:
            tiles[0] = after(tiles[0], v)
        return _cat([_b16(u) for u in tiles])

    def put_pair(a, h):
        put(lhs32, a, h // 2 * 3, (h - first[group[h]]) // 2 * 3)

    def pair_rows(h):
        return pl.ds(h * (_DH // 2), _DH)

    tm = 0.0
    h_q = 0
    for g, n in enumerate(_GROUPS):
        h0, nt = first[g], n * _DH // _L
        g_next = min(g + 1, len(_GROUPS) - 1)
        while h_q < first[g_next] + _GROUPS[g_next]:
            def q_job(h=h_q):
                w = _cat([_b16(wq32[i]) for i in range(h // 2 * 3, h // 2 * 3 + 3)])
                q = q_dot(w) if h < 4 else _dot(xn, w)
                put_pair(q * _QSCALE, h)
                return q
            tm = mxu(tm, 3 * nd * _T_TILE, q_job)
            t_q[h_q] = tm + 150
            h_q += 2
        tm = max(tm, t_q[h0 + n - 2])
        for c in range(nc):
            for i in range(0, nt, 3):
                def qk_job(g=g, h0=h0, nt=nt, c=c, i=i, tm=tm):
                    rows = pl.ds((h0 * _DH + i * _L) // 2, 3 * _L // 2)
                    s = _dot(lhs_tiles(lhs32, h0 // 2 * 3 + i, 3, tm), _b16(k32[c, rows, :]))
                    st["s"] = s = st["s"] + s if i else s
                    if i + 3 == nt:
                        s_ref[g % 2, c] = s
                    return s
                tm = mxu(tm, 3 * _T_TILE, qk_job)

        t = tm + _T_MXU

        def row_max(g=g, t=t):
            m = _tree([s_ref[g % 2, c] for c in range(nc)], jnp.maximum)
            st["m", g] = jnp.broadcast_to(jnp.max(m, axis=-1, keepdims=True), (8, _L))
            results.append((t + _T_MAX, st["m", g]))
        at(t, row_max)
        for c0 in range(0, nc, 8):
            def exps(g=g, c0=c0, t=t):
                ps = [jnp.exp2(s_ref[g % 2, c] - st["m", g]) for c in range(c0, c0 + 8)]
                for c, p in zip(range(c0, c0 + 8), ps):
                    if first[g] < h_vpu:
                        p_ref[g, c] = p
                    if g == group[-1]:
                        p16[c] = _lhs(p)
                st["l", g] = _tree(ps + ([st["l", g]] if c0 else []))
                results.append((t + _T_MAX + 40 + 3 * c0, st["l", g]))
            at(t + min(_T_MAX + 3 * c0, _T_SOFTMAX - 1), exps)

        def row_sum(g=g):
            inv_l[g] = jnp.broadcast_to(1.0 / jnp.sum(st["l", g], axis=-1, keepdims=True), (8, _L))
        at(t + _T_MAX + 3 * nc + 40, row_sum)
        t_soft[g] = t + _T_SOFTMAX

    tv = 0.0
    for h in range(h_vpu):
        g = group[h]
        n = nc if h < _H_MXU else _C_SPLIT
        early = min(60, max(0, tv - t_soft[g]))
        tv = max(tv, t_soft[g])

        def spread_p(h=h, g=g, n=n):
            for c in range(n):
                p_row[h % 2, c] = jnp.broadcast_to(p_ref[g, c, pl.ds(h - first[g], 1), :], (8, _L))
        at(tv - early, spread_p)
        for r0 in range(0, _DH // 16, _R_BLOCK):
            for c0 in range(0, n, _C_BLOCK):
                c3 = c0 + _C_BLOCK
                c1 = c0 + sum(h < _H_MXU and c in _WIDE for c in range(c0, c3))
                c2 = c3 - 3

                def load_p(h=h, c0=c0, c1=c1, c2=c2, c3=c3):
                    p = p_row.at[h % 2]
                    st["p"] = (p[c0:c1] if c1 > c0 else None, p[c1:c2], [p[c] for c in range(c2, c3)])
                at(tv, load_p)
                for r in range(r0, r0 + _R_BLOCK):
                    def pv_step(h=h, n=n, c0=c0, c1=c1, c2=c2, c3=c3, r=r, tv=tv):
                        rows = pl.ds(h * (_DH // 2) + r * 8, 8)
                        p_wide, p_mid, p_end = st["p"]
                        w = v32[c1:c2, rows, :]
                        lo = jnp.sum(pltpu.bitcast(w << 16, f32) * p_mid, axis=0)
                        hi = jnp.sum(pltpu.bitcast(w & _HI, f32) * p_mid, axis=0)
                        more = [st[r]] if c0 else []
                        if c1 > c0:
                            e = _WIDE.index(c0)
                            more.append((
                                jnp.sum(pltpu.bitcast(v_lo[e:e + c1 - c0, rows, :], f32) * p_wide, axis=0),
                                jnp.sum(pltpu.bitcast(v32[c0:c1, rows, :], f32) * p_wide, axis=0)))
                        if more:
                            lo, hi = lo + _tree([u[0] for u in more]), hi + _tree([u[1] for u in more])
                        for c, p in zip(range(c2, c3), p_end):
                            w = v32[c, rows, :]
                            if c == c2:
                                for _, v in steps[-1:]:
                                    w = after(w, v)
                                for t, v in results:
                                    if t_soft[0] + 50 < t <= tv:
                                        w = after(w, v)
                                results[:] = [u for u in results if u[0] > tv]
                            lo = lo + pltpu.bitcast(w << 16, f32) * p
                            hi = hi + pltpu.bitcast(w & _HI, f32) * p
                        st[r] = (lo, hi)
                        if c3 < n:
                            done = after(hi, lo)
                        else:
                            done = pltpu.bitcast(
                                pltpu.pack_elementwise([lo, hi], packed_dtype=bf16), i32)
                            v32[0, rows, :] = done
                        steps[:] = steps[-100:] + [(tv, done)]
                    at(tv, pv_step)
                    tv += (4 * (c1 - c0) + 6 * (c3 - c1) + 2) * _T_VOP
        t_head[h] = tv

    c_first = {h: _C_SPLIT if h < h_vpu else 0 for h in range(_H_MXU, _HQ, 2)}
    todo_sum = list(range(0, h_vpu, 2))
    todo_pv = [(h, c) for h in range(_H_MXU, _HQ, 2) for c in range(c_first[h], nc, 2)]
    todo_out = []
    while todo_sum or todo_pv or todo_out:
        if (todo_sum and t_head[todo_sum[0] + 1] + 30 <= tm
                and all(u[0] > todo_sum[0] for u in todo_pv)):
            h = todo_sum.pop(0)

            def sum_job(h=h):
                o = _dot_nt(ones, _b16(v32[0, pair_rows(h), :]))
                if h == _H_MXU:
                    o = o + o_acc[0, :, 0:2 * _DH]
                put_pair(o * _cat([inv_l[group[h]]] * 3), h)
                return o
            tm = mxu(tm, 6 * _T_TILE, sum_job)
            todo_out.append((tm + _T_MXU, h))
        elif todo_pv and t_soft[group[-1]] <= tm and (len(todo_out) <= 2 or todo_out[0][0] > tm):
            h, c0 = todo_pv.pop(0)

            def pv_job(h=h, c0=c0, tm=tm):
                for c in (c0, c0 + 1):
                    v = [v32[c, pl.ds((h * _DH + i * _L) // 2, _L // 2), :] for i in range(3)]
                    o = _dot(lhs_tiles(p16_32, c, 1, tm if c == c0 else -1),
                             _cat([_b16(u) for u in v]))
                    st["s"] = st["s"] + o if c > c_first[h] else o
                if c0 + 2 == nc and h < h_vpu:
                    o_acc[0, :, 0:2 * _DH] = st["s"]
                elif c0 + 2 == nc:
                    put_pair(st["s"] * _cat([inv_l[group[h]]] * 3), h)
                return st["s"]
            tm = mxu(tm, 6 * _T_TILE, pv_job)
            if c0 + 2 == nc and h >= h_vpu:
                todo_out.append((tm + _T_MXU, h))
        elif todo_out and todo_out[0][0] <= tm:
            def out_job(h=todo_out.pop(0)[1], tm=tm):
                y = _dot(lhs_tiles(lhs32, h // 2 * 3, 3, tm),
                         _cat([_b16(wo32[i, pair_rows(h), :]) for i in range(nd)]))
                st["out"] = st["out"] + y if "out" in st else y
                return st["out"]
            tm = mxu(tm, 3 * nd * _T_TILE, out_job)
        else:
            tm += _T_TILE

    for _, _, fn in sorted(events, key=lambda e: e[:2]):
        fn()
    return st["out"]


def _kernel(x_hbm, k_hbm, v_hbm, wq_hbm, wo_hbm, wg_hbm, wu_hbm, wd_hbm, o_ref,
            x_buf, k_buf, v_buf, v_lo, wq, wo, wg, wu, wd, lhs, diag, s_ref, p_ref, p16, p_row,
            inv_l, o_acc, ring, w_sem, *, start):
    nc = k_buf.shape[0]
    d_model = x_buf.shape[-1]
    nd = d_model // _L
    ng = _HQ // 8
    nt = 8 * _DH // _L
    half = 8 * _DH // 2
    assert nc % _RING == 0
    k32, v32, wq32, wo32, lhs32 = (r.bitcast(i32) for r in (k_buf, v_buf, wq, wo, lhs))

    def window_copy(src, dst, c):
        keys = pl.ds(pl.multiple_of(start + c * _L, _L), _L)
        return pltpu.make_async_copy(src.at[:, keys], dst.at[c], ring.at[c % _RING])

    k_copy = functools.partial(window_copy, k_hbm, k_buf)
    v_copy = functools.partial(window_copy, v_hbm, v_buf)
    x_copy = pltpu.make_async_copy(x_hbm, x_buf, ring.at[_RING - 1])
    cut = wd.shape[0] - 2 * _L
    wd_parts = (slice(0, cut), slice(cut, wd.shape[0]))
    glu_copies = [pltpu.make_async_copy(src, dst, ring.at[i]) for i, (src, dst) in enumerate(
        [(wg_hbm, wg), (wu_hbm, wu)] + [(wd_hbm.at[f], wd.at[f]) for f in wd_parts])]

    def put(ref32, a, t0=0, d0=0):
        a = pltpu.bitcast(_lhs(a), i32)
        for t in range(a.shape[1] // _L):
            ref32[t0 + t] = a[:, t * _L:(t + 1) * _L] & diag[d0 + t]

    x_copy.start()
    k_copy(0).start()

    @pl.loop(0, wq.shape[0])
    def _(t):
        cols = pl.ds(pl.multiple_of(t * _L, _L), _L)
        pltpu.make_async_copy(wq_hbm.at[:, cols], wq.at[t], w_sem.at[0]).start()

    for c in range(1, _RING - 1):
        k_copy(c).start()

    for t in range(nt):
        col = jax.lax.broadcasted_iota(i32, (8, _L), 1) + t * _L
        col = col - jax.lax.broadcasted_iota(i32, (8, _L), 0) * (2 * _DH)
        diag[t] = jnp.where((col >= 0) & (col < 2 * _DH), jnp.where(col < _DH, 0xFFFF, _HI), 0)
    o_acc[...] = jnp.zeros(o_acc.shape, f32)
    x_copy.wait()
    k_copy(_RING - 1).start()
    pltpu.make_async_copy(wq, wq, w_sem.at[0]).wait()
    x = jnp.broadcast_to(x_buf[0].astype(f32), (8, d_model))
    xn = _layernorm(x)

    @pl.loop(0, ng)
    def _(g):
        w = wq32.at[pl.ds(g * nt, nt)]
        put(lhs32.at[pl.ds(g * nt, nt)], _dot(xn, _cat([_b16(w[t]) for t in range(nt)])) * _QSCALE)

    @pl.loop(0, nc)
    def _(c):
        k_copy(c).wait()
        n = wo.shape[1] // nc
        rows = pl.ds(pl.multiple_of(c * n, n), n)
        for t in range(nd):
            pltpu.make_async_copy(
                wo_hbm.at[rows, pl.ds(t * _L, _L)], wo.at[t, rows], w_sem.at[0]).start()
        pl.when(c + _RING < nc)(lambda: k_copy(c + _RING).start())
        pl.when(c + _RING >= nc)(lambda: v_copy(c + _RING - nc).start())
        for g in range(ng):
            q = _cat([lhs[g * nt + t] for t in range(nt)])
            s_ref[g, c] = _dot(q, _b16(k32[c, pl.ds(g * half, half), :]))

    @pl.loop(0, ng)
    def _(g):
        s = [s_ref[g, c] for c in range(nc)]
        m = jnp.max(_tree(s, jnp.maximum), axis=-1, keepdims=True)
        p = [jnp.exp2(u - m) for u in s]
        inv_l[g] = jnp.broadcast_to(1.0 / jnp.sum(_tree(p), axis=-1, keepdims=True), (8, _L))
        for c in range(nc):
            s_ref[g, c] = p[c]

    def v_step(c, count):
        v_copy(c).wait()
        pl.when(c + _RING < nc)(lambda: v_copy(c + _RING).start())
        for i, cp in enumerate(glu_copies):
            pl.when(c + _RING == nc + i)(cp.start)
        for g in range(ng):
            o_acc[g] += _dot_nt(_lhs(s_ref[g, c]), _b16(v32[c, pl.ds(g * half, half), :]))

        def transpose(h0, h1):
            for r0 in range(h0 * _DH, h1 * _DH, _L):
                v_buf[c, pl.ds(r0, _L), :] = v_buf[c, pl.ds(r0, _L), :].T

        transpose(_H_MXU + 2, _HQ)
        pl.when(c >= _C_SPLIT)(lambda: transpose(_H_MXU, _H_MXU + 2))

        @pl.when(functools.reduce(jnp.logical_or, [c == e for e in _WIDE]))
        def _():
            src = v32.at[c]
            dst = v_lo.at[sum(jnp.where(c == e, i, 0) for i, e in enumerate(_WIDE))]
            for r0 in range(0, _H_MXU * _DH // 2, _DH // 2):
                w = src[pl.ds(r0, _DH // 2), :]
                dst[pl.ds(r0, _DH // 2), :] = w << 16
                src[pl.ds(r0, _DH // 2), :] = w & _HI
        return count + 1

    never = jax.lax.fori_loop(0, nc, v_step, 0) < 0
    pltpu.make_async_copy(wo, wo, w_sem.at[0]).wait()

    def out_step(g, acc):
        put(lhs32, o_acc[g] * _cat([inv_l[g]] * nt))
        w = wo32.at[:, pl.ds(pl.multiple_of(g * half, half), half), :]
        return acc + _dot(_cat([lhs[t] for t in range(nt)]), _cat([_b16(w[t]) for t in range(nd)]))

    x = x + _rowsum(jax.lax.fori_loop(0, ng, out_step, jnp.zeros((8, d_model), f32)))
    xn = _layernorm(x)
    glu_copies[0].wait()
    gate = _dot(xn, wg[...])
    glu_copies[1].wait()
    hidden = _lhs(jax.nn.sigmoid(gate) * _dot(xn, wu[...]))
    for cp, f in zip(glu_copies[2:], wd_parts):
        cp.wait()
        x = x + _dot(hidden[:, f], wd[f, :])

    x = x + _rowsum(_second_attention(
        *_layernorm_dot(x), never, k32, v32, v_lo, wq32, wo32, lhs32, put, s_ref, p_ref, p16,
        p_row, inv_l, o_acc))
    xn_dot, _ = _layernorm_dot(x)
    gate, up = xn_dot(wg[...]), xn_dot(wu[...])
    x = x + _dot(_lhs(jax.nn.sigmoid(gate) * up), wd[...])
    o_ref[0] = x[0:1, :].astype(o_ref.dtype)


@jax.jit
def pallas_interleave_layers__sliding_block_cached__glu_gated_glu__decode_kernel(
    A_x: jax.Array,
    A_k_cache: jax.Array,
    A_v_cache: jax.Array,
    A_wq: jax.Array,
    A_wo: jax.Array,
    B_x: jax.Array,
    B_w_gate: jax.Array,
    B_w_up: jax.Array,
    B_w_down: jax.Array,
):
    del B_x
    _, hkv, sk, dh = A_k_cache.shape
    d_model = A_x.shape[-1]
    window = min(4096, max(256, sk // 4))
    assert A_x.shape[:2] == (1, 1) and (hkv, dh, window) == (_HQ, _DH, 4096) and sk % _L == 0
    nc = window // _L
    hd = hkv * dh

    kt = jnp.transpose(A_k_cache, (0, 1, 3, 2)).reshape(hd, sk)
    vt = jnp.transpose(A_v_cache, (0, 1, 3, 2)).reshape(hd, sk)

    return pl.pallas_call(
        functools.partial(_kernel, start=sk - window),
        out_shape=jax.ShapeDtypeStruct(A_x.shape, A_x.dtype),
        in_specs=[pl.BlockSpec(memory_space=pltpu.HBM)] * 8,
        out_specs=pl.BlockSpec(memory_space=pltpu.VMEM),
        scratch_shapes=[
            pltpu.VMEM(A_x.shape, bf16),
            pltpu.VMEM((nc, hd, _L), bf16),
            pltpu.VMEM((nc, hd, _L), bf16),
            pltpu.VMEM((len(_WIDE), _H_MXU * dh // 2, _L), i32),
            pltpu.VMEM((hd // _L, d_model, _L), bf16),
            pltpu.VMEM((d_model // _L, hd, _L), bf16),
            pltpu.VMEM(B_w_gate.shape, bf16),
            pltpu.VMEM(B_w_up.shape, bf16),
            pltpu.VMEM(B_w_down.shape, bf16),
            pltpu.VMEM((hd // _L, 16, _L), bf16),
            pltpu.VMEM((8 * dh // _L, 8, _L), i32),
            pltpu.VMEM((hkv // 8, nc, 8, _L), f32),
            pltpu.VMEM((len(_GROUPS), nc, 8, _L), f32),
            pltpu.VMEM((nc, 16, _L), bf16),
            pltpu.VMEM((2, nc, 8, _L), f32),
            pltpu.VMEM((len(_GROUPS), 8, _L), f32),
            pltpu.VMEM((hkv // 8, 8, 8 * dh), f32),
            pltpu.SemaphoreType.DMA((_RING,)),
            pltpu.SemaphoreType.DMA((1,)),
        ],
        compiler_params=pltpu.CompilerParams(vmem_limit_bytes=127 * 1024 * 1024),
    )(A_x, kt, vt, A_wq, A_wo, B_w_gate, B_w_up, B_w_down)
```

```python
import functools

import jax
import jax.numpy as jnp
from jax.experimental import pallas as pl
from jax.experimental.pallas import tpu as pltpu

f32, bf16, i32 = jnp.float32, jnp.bfloat16, jnp.int32

_HQ = 32
_DH = 192
_L = 128
_EPS = 1e-5
_QSCALE = (_DH ** -0.5) * 1.4426950408889634
_HI = -65536
_RING = 4

_GROUPS = (2, 2, 4, 4, 6, 8, 6)
_H_MXU = 26
_C_SPLIT = 16
_C_BLOCK = 8
_R_BLOCK = 4
_WIDE = (0, 1, 8, 9, 16, 24)
_T_TILE = 8
_T_VOP = 0.275
_T_MXU = 200
_T_MAX = 170
_T_SOFTMAX = 200


def _cat(xs):
    return xs[0] if len(xs) == 1 else jnp.concatenate(xs, axis=1)


def _tree(xs, op=jnp.add):
    while len(xs) > 1:
        xs = [op(xs[i], xs[i + 1]) if i + 1 < len(xs) else xs[i] for i in range(0, len(xs), 2)]
    return xs[0]


def _b16(w):
    return pltpu.bitcast(w, bf16)


def _lhs(a):
    return jnp.concatenate([a, jnp.zeros_like(a)], axis=0).astype(bf16)


def _dot(a, b):
    return jnp.dot(a, b, preferred_element_type=f32)[0:8]


def _dot_nt(a, b):
    return jax.lax.dot_general(a, b, (((1,), (1,)), ((), ())), preferred_element_type=f32)[0:8]


def _rowsum(a):
    return jnp.broadcast_to(jnp.sum(a, axis=0, keepdims=True), a.shape)


def _ln_stats(x):
    m = jnp.mean(x, axis=-1, keepdims=True)
    d = x - m
    return m, d, jax.lax.rsqrt(jnp.mean(d * d, axis=-1, keepdims=True) + _EPS)


def _layernorm(x):
    _, d, r = _ln_stats(x)
    return _lhs(d * r)


def _layernorm_dot(x):
    m, d, r = _ln_stats(x)
    x_ones = jnp.concatenate([x, jnp.ones_like(x)], axis=0).astype(bf16)

    def f(w):
        y = jnp.dot(x_ones, w, preferred_element_type=f32)
        return (y[0:8] - m * y[8:16]) * r

    return f, _lhs(d * r)


def _second_attention(q_dot, xn, never, k32, v32, v_lo, wq32, wo32, lhs32, put, s_ref, p_ref, p16,
                      p_row, inv_l, o_acc):
    nc, nd = k32.shape[0], wo32.shape[0]
    p16_32 = p16.bitcast(i32)
    h_vpu = _H_MXU + 2
    first = [sum(_GROUPS[:g]) for g in range(len(_GROUPS))]
    group = [g for g, n in enumerate(_GROUPS) for _ in range(n)]
    assert len(group) == _HQ and group[_H_MXU] == group[-1] and _C_SPLIT < nc
    ones = jnp.ones((16, _L), bf16)
    events = []
    results = []
    steps = []
    st = {}
    t_q, t_soft, t_head = {}, {}, {}

    def after(a, dep):
        return jnp.where(never, pltpu.bitcast(dep, a.dtype), a)

    def at(t, fn):
        events.append((t, len(events), fn))

    def mxu(t, cycles, fn):
        def run():
            r = fn()
            results.append((t + cycles + _T_MXU, r[:, r.shape[1] - _L:]))
        at(t, run)
        return t + cycles

    def lhs_tiles(ref32, t0, n, t):
        tiles = [ref32[i] for i in range(t0, t0 + n)]
        for v in [v for (tv, v) in steps if tv <= t][-1:]:
            tiles[0] = after(tiles[0], v)
        return _cat([_b16(u) for u in tiles])

    def put_pair(a, h):
        put(lhs32, a, h // 2 * 3, (h - first[group[h]]) // 2 * 3)

    def pair_rows(h):
        return pl.ds(h * (_DH // 2), _DH)

    tm = 0.0
    h_q = 0
    for g, n in enumerate(_GROUPS):
        h0, nt = first[g], n * _DH // _L
        g_next = min(g + 1, len(_GROUPS) - 1)
        while h_q < first[g_next] + _GROUPS[g_next]:
            def q_job(h=h_q):
                w = _cat([_b16(wq32[i]) for i in range(h // 2 * 3, h // 2 * 3 + 3)])
                q = q_dot(w) if h < 4 else _dot(xn, w)
                put_pair(q * _QSCALE, h)
                return q
            tm = mxu(tm, 3 * nd * _T_TILE, q_job)
            t_q[h_q] = tm + 150
            h_q += 2
        tm = max(tm, t_q[h0 + n - 2])
        for c in range(nc):
            for i in range(0, nt, 3):
                def qk_job(g=g, h0=h0, nt=nt, c=c, i=i, tm=tm):
                    rows = pl.ds((h0 * _DH + i * _L) // 2, 3 * _L // 2)
                    s = _dot(lhs_tiles(lhs32, h0 // 2 * 3 + i, 3, tm), _b16(k32[c, rows, :]))
                    st["s"] = s = st["s"] + s if i else s
                    if i + 3 == nt:
                        s_ref[g % 2, c] = s
                    return s
                tm = mxu(tm, 3 * _T_TILE, qk_job)

        t = tm + _T_MXU

        def row_max(g=g, t=t):
            m = _tree([s_ref[g % 2, c] for c in range(nc)], jnp.maximum)
            st["m", g] = jnp.broadcast_to(jnp.max(m, axis=-1, keepdims=True), (8, _L))
            results.append((t + _T_MAX, st["m", g]))
        at(t, row_max)
        for c0 in range(0, nc, 8):
            def exps(g=g, c0=c0, t=t):
                ps = [jnp.exp2(s_ref[g % 2, c] - st["m", g]) for c in range(c0, c0 + 8)]
                for c, p in zip(range(c0, c0 + 8), ps):
                    if first[g] < h_vpu:
                        p_ref[g, c] = p
                    if g == group[-1]:
                        p16[c] = _lhs(p)
                st["l", g] = _tree(ps + ([st["l", g]] if c0 else []))
                results.append((t + _T_MAX + 40 + 3 * c0, st["l", g]))
            at(t + min(_T_MAX + 3 * c0, _T_SOFTMAX - 1), exps)

        def row_sum(g=g):
            inv_l[g] = jnp.broadcast_to(1.0 / jnp.sum(st["l", g], axis=-1, keepdims=True), (8, _L))
        at(t + _T_MAX + 3 * nc + 40, row_sum)
        t_soft[g] = t + _T_SOFTMAX

    tv = 0.0
    for h in range(h_vpu):
        g = group[h]
        n = nc if h < _H_MXU else _C_SPLIT
        early = min(60, max(0, tv - t_soft[g]))
        tv = max(tv, t_soft[g])

        def spread_p(h=h, g=g, n=n):
            for c in range(n):
                p_row[h % 2, c] = jnp.broadcast_to(p_ref[g, c, pl.ds(h - first[g], 1), :], (8, _L))
        at(tv - early, spread_p)
        for r0 in range(0, _DH // 16, _R_BLOCK):
            for c0 in range(0, n, _C_BLOCK):
                c3 = c0 + _C_BLOCK
                c1 = c0 + sum(h < _H_MXU and c in _WIDE for c in range(c0, c3))
                c2 = c3 - 3

                def load_p(h=h, c0=c0, c1=c1, c2=c2, c3=c3):
                    p = p_row.at[h % 2]
                    st["p"] = (p[c0:c1] if c1 > c0 else None, p[c1:c2], [p[c] for c in range(c2, c3)])
                at(tv, load_p)
                for r in range(r0, r0 + _R_BLOCK):
                    def pv_step(h=h, n=n, c0=c0, c1=c1, c2=c2, c3=c3, r=r, tv=tv):
                        rows = pl.ds(h * (_DH // 2) + r * 8, 8)
                        p_wide, p_mid, p_end = st["p"]
                        w = v32[c1:c2, rows, :]
                        lo = jnp.sum(pltpu.bitcast(w << 16, f32) * p_mid, axis=0)
                        hi = jnp.sum(pltpu.bitcast(w & _HI, f32) * p_mid, axis=0)
                        more = [st[r]] if c0 else []
                        if c1 > c0:
                            e = _WIDE.index(c0)
                            more.append((
                                jnp.sum(pltpu.bitcast(v_lo[e:e + c1 - c0, rows, :], f32) * p_wide, axis=0),
                                jnp.sum(pltpu.bitcast(v32[c0:c1, rows, :], f32) * p_wide, axis=0)))
                        if more:
                            lo, hi = lo + _tree([u[0] for u in more]), hi + _tree([u[1] for u in more])
                        for c, p in zip(range(c2, c3), p_end):
                            w = v32[c, rows, :]
                            if c == c2:
                                for _, v in steps[-1:]:
                                    w = after(w, v)
                                for t, v in results:
                                    if t_soft[0] + 50 < t <= tv:
                                        w = after(w, v)
                                results[:] = [u for u in results if u[0] > tv]
                            lo = lo + pltpu.bitcast(w << 16, f32) * p
                            hi = hi + pltpu.bitcast(w & _HI, f32) * p
                        st[r] = (lo, hi)
                        if c3 < n:
                            done = after(hi, lo)
                        else:
                            done = pltpu.bitcast(jnp.concatenate([lo, hi], axis=0).astype(bf16), i32)
                            v32[0, rows, :] = done
                        steps[:] = steps[-100:] + [(tv, done)]
                    at(tv, pv_step)
                    tv += (4 * (c1 - c0) + 6 * (c3 - c1) + 2) * _T_VOP
        t_head[h] = tv

    c_first = {h: _C_SPLIT if h < h_vpu else 0 for h in range(_H_MXU, _HQ, 2)}
    todo_sum = list(range(0, h_vpu, 2))
    todo_pv = [(h, c) for h in range(_H_MXU, _HQ, 2) for c in range(c_first[h], nc, 2)]
    todo_out = []
    while todo_sum or todo_pv or todo_out:
        if (todo_sum and t_head[todo_sum[0] + 1] + 30 <= tm
                and all(u[0] > todo_sum[0] for u in todo_pv)):
            h = todo_sum.pop(0)

            def sum_job(h=h):
                o = _dot_nt(ones, _b16(v32[0, pair_rows(h), :]))
                if h == _H_MXU:
                    o = o + o_acc[0, :, 0:2 * _DH]
                put_pair(o * _cat([inv_l[group[h]]] * 3), h)
                return o
            tm = mxu(tm, 6 * _T_TILE, sum_job)
            todo_out.append((tm + _T_MXU, h))
        elif todo_pv and t_soft[group[-1]] <= tm and (len(todo_out) <= 2 or todo_out[0][0] > tm):
            h, c0 = todo_pv.pop(0)

            def pv_job(h=h, c0=c0, tm=tm):
                for c in (c0, c0 + 1):
                    v = [v32[c, pl.ds((h * _DH + i * _L) // 2, _L // 2), :] for i in range(3)]
                    o = _dot(lhs_tiles(p16_32, c, 1, tm if c == c0 else -1),
                             _cat([_b16(u) for u in v]))
                    st["s"] = st["s"] + o if c > c_first[h] else o
                if c0 + 2 == nc and h < h_vpu:
                    o_acc[0, :, 0:2 * _DH] = st["s"]
                elif c0 + 2 == nc:
                    put_pair(st["s"] * _cat([inv_l[group[h]]] * 3), h)
                return st["s"]
            tm = mxu(tm, 6 * _T_TILE, pv_job)
            if c0 + 2 == nc and h >= h_vpu:
                todo_out.append((tm + _T_MXU, h))
        elif todo_out and todo_out[0][0] <= tm:
            def out_job(h=todo_out.pop(0)[1], tm=tm):
                y = _dot(lhs_tiles(lhs32, h // 2 * 3, 3, tm),
                         _cat([_b16(wo32[i, pair_rows(h), :]) for i in range(nd)]))
                st["out"] = st["out"] + y if "out" in st else y
                return st["out"]
            tm = mxu(tm, 3 * nd * _T_TILE, out_job)
        else:
            tm += _T_TILE

    for _, _, fn in sorted(events, key=lambda e: e[:2]):
        fn()
    return st["out"]


def _kernel(x_hbm, k_hbm, v_hbm, wq_hbm, wo_hbm, wg_hbm, wu_hbm, wd_hbm, o_ref,
            x_buf, k_buf, v_buf, v_lo, wq, wo, wg, wu, wd, lhs, diag, s_ref, p_ref, p16, p_row,
            inv_l, o_acc, ring, w_sem, *, start):
    nc = k_buf.shape[0]
    d_model = x_buf.shape[-1]
    nd = d_model // _L
    ng = _HQ // 8
    nt = 8 * _DH // _L
    half = 8 * _DH // 2
    assert nc % _RING == 0
    k32, v32, wq32, wo32, lhs32 = (r.bitcast(i32) for r in (k_buf, v_buf, wq, wo, lhs))

    def window_copy(src, dst, c):
        keys = pl.ds(pl.multiple_of(start + c * _L, _L), _L)
        return pltpu.make_async_copy(src.at[:, keys], dst.at[c], ring.at[c % _RING])

    k_copy = functools.partial(window_copy, k_hbm, k_buf)
    v_copy = functools.partial(window_copy, v_hbm, v_buf)
    x_copy = pltpu.make_async_copy(x_hbm, x_buf, ring.at[_RING - 1])
    cut = wd.shape[0] - 2 * _L
    wd_parts = (slice(0, cut), slice(cut, wd.shape[0]))
    glu_copies = [pltpu.make_async_copy(src, dst, ring.at[i]) for i, (src, dst) in enumerate(
        [(wg_hbm, wg), (wu_hbm, wu)] + [(wd_hbm.at[f], wd.at[f]) for f in wd_parts])]

    def put(ref32, a, t0=0, d0=0):
        a = pltpu.bitcast(_lhs(a), i32)
        for t in range(a.shape[1] // _L):
            ref32[t0 + t] = a[:, t * _L:(t + 1) * _L] & diag[d0 + t]

    x_copy.start()
    k_copy(0).start()

    @pl.loop(0, wq.shape[0])
    def _(t):
        cols = pl.ds(pl.multiple_of(t * _L, _L), _L)
        pltpu.make_async_copy(wq_hbm.at[:, cols], wq.at[t], w_sem.at[0]).start()

    for c in range(1, _RING - 1):
        k_copy(c).start()

    for t in range(nt):
        col = jax.lax.broadcasted_iota(i32, (8, _L), 1) + t * _L
        col = col - jax.lax.broadcasted_iota(i32, (8, _L), 0) * (2 * _DH)
        diag[t] = jnp.where((col >= 0) & (col < 2 * _DH), jnp.where(col < _DH, 0xFFFF, _HI), 0)
    o_acc[...] = jnp.zeros(o_acc.shape, f32)
    x_copy.wait()
    k_copy(_RING - 1).start()
    pltpu.make_async_copy(wq, wq, w_sem.at[0]).wait()
    x = jnp.broadcast_to(x_buf[0].astype(f32), (8, d_model))
    xn = _layernorm(x)

    @pl.loop(0, ng)
    def _(g):
        w = wq32.at[pl.ds(g * nt, nt)]
        put(lhs32.at[pl.ds(g * nt, nt)], _dot(xn, _cat([_b16(w[t]) for t in range(nt)])) * _QSCALE)

    @pl.loop(0, nc)
    def _(c):
        k_copy(c).wait()
        n = wo.shape[1] // nc
        rows = pl.ds(pl.multiple_of(c * n, n), n)
        for t in range(nd):
            pltpu.make_async_copy(
                wo_hbm.at[rows, pl.ds(t * _L, _L)], wo.at[t, rows], w_sem.at[0]).start()
        pl.when(c + _RING < nc)(lambda: k_copy(c + _RING).start())
        pl.when(c + _RING >= nc)(lambda: v_copy(c + _RING - nc).start())
        for g in range(ng):
            q = _cat([lhs[g * nt + t] for t in range(nt)])
            s_ref[g, c] = _dot(q, _b16(k32[c, pl.ds(g * half, half), :]))

    @pl.loop(0, ng)
    def _(g):
        s = [s_ref[g, c] for c in range(nc)]
        m = jnp.max(_tree(s, jnp.maximum), axis=-1, keepdims=True)
        p = [jnp.exp2(u - m) for u in s]
        inv_l[g] = jnp.broadcast_to(1.0 / jnp.sum(_tree(p), axis=-1, keepdims=True), (8, _L))
        for c in range(nc):
            s_ref[g, c] = p[c]

    def v_step(c, count):
        v_copy(c).wait()
        pl.when(c + _RING < nc)(lambda: v_copy(c + _RING).start())
        for i, cp in enumerate(glu_copies):
            pl.when(c + _RING == nc + i)(cp.start)
        for g in range(ng):
            o_acc[g] += _dot_nt(_lhs(s_ref[g, c]), _b16(v32[c, pl.ds(g * half, half), :]))

        def transpose(h0, h1):
            for r0 in range(h0 * _DH, h1 * _DH, _L):
                v_buf[c, pl.ds(r0, _L), :] = v_buf[c, pl.ds(r0, _L), :].T

        def repack(h0, h1, lo_ref=None):
            for r in range(h0 * _DH // 16, h1 * _DH // 16):
                rows = pl.ds(r * 8, 8)
                w = pltpu.bitcast(_b16(v32[c, rows, :]).astype(f32), i32)
                if lo_ref is None:
                    v32[c, rows, :] = jax.lax.shift_right_logical(w[0:8], 16) | w[8:16]
                else:
                    lo_ref[rows, :] = w[0:8]
                    v32[c, rows, :] = w[8:16]

        transpose(_H_MXU + 2, _HQ)
        pl.when(c >= _C_SPLIT)(lambda: transpose(_H_MXU, _H_MXU + 2))
        pl.when(c < _C_SPLIT)(lambda: repack(_H_MXU, _H_MXU + 2))
        wide = functools.reduce(jnp.logical_or, [c == e for e in _WIDE])
        slot = sum(jnp.where(c == e, i, 0) for i, e in enumerate(_WIDE))
        pl.when(wide)(lambda: repack(0, _H_MXU, v_lo.at[slot]))
        pl.when(jnp.logical_not(wide))(lambda: repack(0, _H_MXU))
        return count + 1

    never = jax.lax.fori_loop(0, nc, v_step, 0) < 0
    pltpu.make_async_copy(wo, wo, w_sem.at[0]).wait()

    def out_step(g, acc):
        put(lhs32, o_acc[g] * _cat([inv_l[g]] * nt))
        w = wo32.at[:, pl.ds(pl.multiple_of(g * half, half), half), :]
        return acc + _dot(_cat([lhs[t] for t in range(nt)]), _cat([_b16(w[t]) for t in range(nd)]))

    x = x + _rowsum(jax.lax.fori_loop(0, ng, out_step, jnp.zeros((8, d_model), f32)))
    xn = _layernorm(x)
    glu_copies[0].wait()
    gate = _dot(xn, wg[...])
    glu_copies[1].wait()
    hidden = _lhs(jax.nn.sigmoid(gate) * _dot(xn, wu[...]))
    for cp, f in zip(glu_copies[2:], wd_parts):
        cp.wait()
        x = x + _dot(hidden[:, f], wd[f, :])

    x = x + _rowsum(_second_attention(
        *_layernorm_dot(x), never, k32, v32, v_lo, wq32, wo32, lhs32, put, s_ref, p_ref, p16,
        p_row, inv_l, o_acc))
    xn_dot, _ = _layernorm_dot(x)
    gate, up = xn_dot(wg[...]), xn_dot(wu[...])
    x = x + _dot(_lhs(jax.nn.sigmoid(gate) * up), wd[...])
    o_ref[0] = x[0:1, :].astype(o_ref.dtype)


@jax.jit
def pallas_interleave_layers__sliding_block_cached__glu_gated_glu__decode_kernel(
    A_x: jax.Array,
    A_k_cache: jax.Array,
    A_v_cache: jax.Array,
    A_wq: jax.Array,
    A_wo: jax.Array,
    B_x: jax.Array,
    B_w_gate: jax.Array,
    B_w_up: jax.Array,
    B_w_down: jax.Array,
):
    del B_x
    _, hkv, sk, dh = A_k_cache.shape
    d_model = A_x.shape[-1]
    window = min(4096, max(256, sk // 4))
    assert A_x.shape[:2] == (1, 1) and (hkv, dh, window) == (_HQ, _DH, 4096) and sk % _L == 0
    nc = window // _L
    hd = hkv * dh

    kt = jnp.transpose(A_k_cache, (0, 1, 3, 2)).reshape(hd, sk)
    vt = jnp.transpose(A_v_cache, (0, 1, 3, 2)).reshape(hd, sk)

    return pl.pallas_call(
        functools.partial(_kernel, start=sk - window),
        out_shape=jax.ShapeDtypeStruct(A_x.shape, A_x.dtype),
        in_specs=[pl.BlockSpec(memory_space=pltpu.HBM)] * 8,
        out_specs=pl.BlockSpec(memory_space=pltpu.VMEM),
        scratch_shapes=[
            pltpu.VMEM(A_x.shape, bf16),
            pltpu.VMEM((nc, hd, _L), bf16),
            pltpu.VMEM((nc, hd, _L), bf16),
            pltpu.VMEM((len(_WIDE), _H_MXU * dh // 2, _L), i32),
            pltpu.VMEM((hd // _L, d_model, _L), bf16),
            pltpu.VMEM((d_model // _L, hd, _L), bf16),
            pltpu.VMEM(B_w_gate.shape, bf16),
            pltpu.VMEM(B_w_up.shape, bf16),
            pltpu.VMEM(B_w_down.shape, bf16),
            pltpu.VMEM((hd // _L, 16, _L), bf16),
            pltpu.VMEM((8 * dh // _L, 8, _L), i32),
            pltpu.VMEM((hkv // 8, nc, 8, _L), f32),
            pltpu.VMEM((len(_GROUPS), nc, 8, _L), f32),
            pltpu.VMEM((nc, 16, _L), bf16),
            pltpu.VMEM((2, nc, 8, _L), f32),
            pltpu.VMEM((len(_GROUPS), 8, _L), f32),
            pltpu.VMEM((hkv // 8, 8, 8 * dh), f32),
            pltpu.SemaphoreType.DMA((_RING,)),
            pltpu.SemaphoreType.DMA((1,)),
        ],
        compiler_params=pltpu.CompilerParams(vmem_limit_bytes=127 * 1024 * 1024),
    )(A_x, kt, vt, A_wq, A_wo, B_w_gate, B_w_up, B_w_down)
```
